```python
import jax
import jax.numpy as jnp

def _softmax(x, axis=-1):
    return jax.nn.softmax(x, axis=axis)
def _gelu(x):
    return jax.nn.gelu(x, approximate=True)
def _silu(x):
    return jax.nn.silu(x)
def _sigmoid(x):
    return jax.nn.sigmoid(x)
def _layernorm(x, axis=-1, eps=1e-5):
    m = jnp.mean(x, axis=axis, keepdims=True)
    v = jnp.var(x, axis=axis, keepdims=True)
    return (x - m) / jnp.sqrt(v + eps)
def _scatter_add(tgt, idx, src, axis=0):
    return tgt.at[idx].add(src)
def _segment_sum(src, seg, n):
    return jax.ops.segment_sum(src, seg, n)
class _Rng:
    def __init__(self, key):
        self._k = key
    def _next(self):
        self._k, sub = jax.random.split(self._k)
        return sub
    def normal(self, shape):
        return jax.random.normal(self._next(), shape, dtype=jnp.bfloat16)
    def randint(self, lo, hi, shape):
        return jax.random.randint(self._next(), shape, lo, hi, dtype=jnp.int32)
    def uniform(self, shape, lo=0.0, hi=1.0):
        return jax.random.uniform(self._next(), shape, jnp.bfloat16, lo, hi)
    def permutation(self, n):
        return jax.random.permutation(self._next(), n)


kernel_name = 'interleave_layers__ssm_conv_h3__mixer_s_mlp__prompt'

def setup_inputs():
    _rng = _Rng(jax.random.key(int.from_bytes(__import__("os").urandom(4), "little")))
    _w = (lambda a: (lambda t: t.astype(jnp.bfloat16) if jnp.issubdtype(t.dtype, jnp.floating) else t)(jnp.asarray(a)))
    def _A_setup():
        B, S, D = 1, 2048, 1024
        ks = 4
        return {
            "q": _w((lambda *s: _rng.normal(s) * 0.05)(B, S, D)),
            "k": _w((lambda *s: _rng.normal(s) * 0.05)(B, S, D)),
            "v": _w((lambda *s: _rng.normal(s) * 0.05)(B, S, D)),
            "shift_k": _w((lambda *s: _rng.normal(s) * 0.05)(D, ks) * 0.5),
            "ssm_k": _w((lambda *s: _rng.normal(s) * 0.05)(D, S) * (1.0 / S ** 0.5)),
            "ssm_D": _w((lambda *s: _rng.normal(s) * 0.05)(D)),
        }
    _A_in = _A_setup()

    def _B_setup():
        B, S, D, F = 1, 2048, 1024, 3584
        return {
            "x":  _w((lambda *s: _rng.normal(s) * 0.05)(B, S, D)),
            "w1": _w((lambda *s: _rng.normal(s) * 0.05)(D, D) * (D ** -0.5)),
            "w2": _w((lambda *s: _rng.normal(s) * 0.05)(D, D) * (D ** -0.5)),
            "w3": _w((lambda *s: _rng.normal(s) * 0.05)(D, F) * (D ** -0.5)),
            "w4": _w((lambda *s: _rng.normal(s) * 0.05)(F, D) * (F ** -0.5)),
        }
    _B_in = _B_setup()

    return {
        "A_q": _A_in["q"],
        "A_k": _A_in["k"],
        "A_v": _A_in["v"],
        "A_shift_k": _A_in["shift_k"],
        "A_ssm_k": _A_in["ssm_k"],
        "A_ssm_D": _A_in["ssm_D"],
        "B_x": _B_in["x"],
        "B_w1": _B_in["w1"],
        "B_w2": _B_in["w2"],
        "B_w3": _B_in["w3"],
        "B_w4": _B_in["w4"],
    }

def reference(A_q, A_k, A_v, A_shift_k, A_ssm_k, A_ssm_D, B_x, B_w1, B_w2, B_w3, B_w4):
    def _A_ref(q, k, v, shift_k, ssm_k, ssm_D):
        B, S, D = q.shape
        ks = shift_k.shape[-1]
        k_pad = jnp.pad(k, ((0, 0), (ks - 1, 0), (0, 0)))
        k_shift = jnp.zeros_like(k)
        for t in range(ks):
            k_shift = k_shift + k_pad[:, t:t + S, :] * shift_k[:, ks - 1 - t][None, None, :]
        kv = k_shift * v
        L = 2 * S
        kv_pad = jnp.pad(kv, ((0, 0), (0, S), (0, 0)))
        kf_pad = jnp.pad(ssm_k, ((0, 0), (0, S)))
        kv_f = (lambda x, axes=(-2,-1): jnp.fft.rfft2(x.astype(jnp.float32), axes=axes))(kv_pad[:, None, :, :], axes=(1, 2))
        kf_f = (lambda x, axes=(-2,-1): jnp.fft.rfft2(x.astype(jnp.float32), axes=axes))(kf_pad[:, None, :], axes=(1, 2))
        kf_f = (lambda x, *d: x.transpose(*d))(kf_f, 1, 2, 0)
        y_f = kv_f * kf_f[None, :, :, :]
        y = (lambda x, s, axes=(-2,-1): jnp.fft.irfft2(x, s=s, axes=axes).astype(jnp.bfloat16))(y_f, (1, L), axes=(1, 2))[:, 0, :S, :]
        y = y + kv * ssm_D[None, None, :]
        return q * y

    def _B_ref(x, w1, w2, w3, w4):
        B, S, D = x.shape
        h = _gelu(_layernorm(x, axis=-1) @ w1)
        c = D // 4
        g0 = jnp.pad(h[:, :, 0*c:1*c], ((0, 0), (1, 0), (0, 0)))[:, :S, :]
        g1 = jnp.pad(h[:, :, 1*c:2*c], ((0, 0), (0, 1), (0, 0)))[:, 1:, :]
        g2 = jnp.pad(h[:, :, 2*c:3*c], ((0, 0), (2, 0), (0, 0)))[:, :S, :]
        g3 = jnp.pad(h[:, :, 3*c:   ], ((0, 0), (0, 2), (0, 0)))[:, 2:, :]
        hs = jnp.concatenate([g0, g1, g2, g3], axis=-1) @ w2
        x1 = x + hs
        h2 = _gelu(_layernorm(x1, axis=-1) @ w3) @ w4
        return x1 + h2

    x = A_q
    x = x + _A_ref(_layernorm(x, axis=-1), A_k, A_v, A_shift_k, A_ssm_k, A_ssm_D)
    x = x + _B_ref(_layernorm(x, axis=-1), B_w1, B_w2, B_w3, B_w4)
    x = x + _A_ref(_layernorm(x, axis=-1), A_k, A_v, A_shift_k, A_ssm_k, A_ssm_D)
    x = x + _B_ref(_layernorm(x, axis=-1), B_w1, B_w2, B_w3, B_w4)
    return x
```

```python
import functools

import jax
import jax.numpy as jnp
import numpy as np
import jax.experimental.pallas as pl
import jax.experimental.pallas.tpu as pltpu
from jax import lax

S, D, F = 2048, 1024, 3584
KS = 4
N = 2 * S
N1, N2 = 128, 32
CW = 256
NT = D // CW
G = CW // 128
P = 40
U1 = 2
U2 = 1
TM = 256
FC = 512
EPS = 1e-5
BF = jnp.bfloat16
F32 = jnp.float32


def _dft_constants():
    a = np.arange(N1 // 2)
    k1 = np.arange(N1 // 2)
    b = np.arange(N2)
    ang = -2 * np.pi * np.outer(k1 + 0.5, a) * N2 / N
    f1 = np.empty((N1, N1 // 2))
    f1[0::2], f1[1::2] = np.cos(ang), np.sin(ang)
    g1 = (2.0 / N) * f1.T
    grp = 64 // N2
    f2 = np.zeros((N1 // 2 // grp, 128, 128))
    for k in range(N1 // 2):
        an = -2 * np.pi * np.outer(k + 0.5 + N1 * b, b) / N
        c, s = np.cos(an), np.sin(an)
        p, g = divmod(k, grp)
        r, c0 = g * N2, g * 2 * N2
        f2[p, r:r + N2, c0:c0 + N2] = c
        f2[p, r:r + N2, c0 + N2:c0 + 2 * N2] = -s
        f2[p, 64 + r:64 + r + N2, c0:c0 + N2] = s
        f2[p, 64 + r:64 + r + N2, c0 + N2:c0 + 2 * N2] = c
    g2 = f2.transpose(0, 2, 1)
    return [np.ascontiguousarray(m).astype(np.float32) for m in (f1, f2, g2, g1)]


def _ln(x):
    m = jnp.mean(x, axis=-1, keepdims=True)
    c = x - m
    v = jnp.mean(c * c, axis=-1, keepdims=True)
    return c * lax.rsqrt(v + EPS)


def _gelu(x):
    inner = x * (0.7978845608028654 + 0.7978845608028654 * 0.044715 * (x * x))
    hx = 0.5 * x
    return hx + hx * jnp.tanh(inner)


def _dot(a, b):
    return jnp.dot(a, b, preferred_element_type=F32)


def _kernel(q_hbm, k_hbm, v_hbm, sk_ref, h_hbm, d_ref, f1_ref, f2_ref, g2_ref,
            g1_ref, w1_hbm, w2_hbm, w3_hbm, w4_hbm, o_hbm,
            qbuf, w1, w2, w3, w4, ybuf, csem, wsem, osem):
    def col_copies(j, kbuf, vbuf, hbuf):
        cols = pl.ds(j * CW, CW)
        return (
            pltpu.make_async_copy(k_hbm.at[0, :, cols], kbuf.at[j], csem.at[0, j]),
            pltpu.make_async_copy(v_hbm.at[0, :, cols], vbuf.at[j], csem.at[1, j]),
            pltpu.make_async_copy(h_hbm.at[cols, :], hbuf.at[j], csem.at[2, j]),
        )

    big = (
        pltpu.make_async_copy(q_hbm.at[0], qbuf, wsem.at[0]),
        pltpu.make_async_copy(w1_hbm, w1, wsem.at[1]),
        pltpu.make_async_copy(w2_hbm, w2, wsem.at[2]),
        pltpu.make_async_copy(w3_hbm, w3, wsem.at[3]),
        pltpu.make_async_copy(w4_hbm, w4, wsem.at[4]),
    )

    def conv_phase(kbuf, vbuf, hbuf, kpad, uh, mid, skt):
        for j in range(NT):
            for c in col_copies(j, kbuf, vbuf, hbuf):
                c.start()
        for c in big:
            c.start()
        eye = (lax.broadcasted_iota(jnp.int32, (16, KS), 0)
               == lax.broadcasted_iota(jnp.int32, (16, KS), 1)).astype(BF)
        for j in range(NT):
            skt[j, 0:16, :] = lax.dot_general(
                eye, sk_ref[j * CW:(j + 1) * CW, :], (((1,), (1,)), ((), ())),
                preferred_element_type=F32)
            skt[j, 16:24, :] = jnp.broadcast_to(
                d_ref[:, j * CW:(j + 1) * CW].astype(F32), (8, CW))
        kpad[0:8, :] = jnp.zeros((8, CW), F32)

        def tile(j, carry):
            for jj in range(NT):
                @pl.when(j == jj)
                def _():
                    for c in col_copies(jj, kbuf, vbuf, hbuf):
                        c.wait()
            RB = 256
            for r in range(S // RB):
                kpad[8 + r * RB:8 + (r + 1) * RB, :] = kbuf[j, r * RB:(r + 1) * RB, :].astype(F32)
            for r in range(S // RB):
                acc = None
                for t in range(KS):
                    term = kpad[8 - t + r * RB:8 - t + (r + 1) * RB, :] * skt[j, t:t + 1, :]
                    acc = term if acc is None else acc + term
                u = acc * vbuf[j, r * RB:(r + 1) * RB, :].astype(F32)
                for g in range(G):
                    for a in range(RB // N2):
                        ra = (r * (RB // N2) + a) * P
                        uh[g, ra:ra + N2, :] = u[a * N2:(a + 1) * N2, g * 128:(g + 1) * 128]
            for r in range(S // 128):
                ht = hbuf[j, :, r * 128:(r + 1) * 128].astype(F32).T
                for g in range(G):
                    for a in range(128 // N2):
                        ra = (r * (128 // N2) + a) * P
                        uh[G + g, ra:ra + N2, :] = ht[a * N2:(a + 1) * N2, g * 128:(g + 1) * 128]

            def s1(b, c):
                x = jnp.concatenate(
                    [uh[g, pl.ds(b, N1 // 2, stride=P), :] for g in range(2 * G)], axis=1)
                r = _dot(f1_ref[...], x.astype(BF))
                for g in range(2 * G):
                    mid[g, pl.ds(b, N1, stride=P), :] = r[:, g * 128:(g + 1) * 128]
                return c
            lax.fori_loop(0, N2, s1, 0, unroll=U1)

            def s2(p, c):
                base = p * (128 // N2 * P)
                rows = [pl.ds(base + i * P, N2) for i in range(128 // N2)]
                m = jnp.concatenate(
                    [jnp.concatenate([mid[g, rr, :] for rr in rows], axis=0)
                     for g in range(2 * G)], axis=1)
                z = _dot(f2_ref[p], m.astype(BF))
                ur, ui = z[0:64, 0:CW], z[64:128, 0:CW]
                hr, hi = z[0:64, CW:], z[64:128, CW:]
                yv = jnp.concatenate([ur * hr - ui * hi, ur * hi + ui * hr], axis=0)
                r = _dot(g2_ref[p], yv.astype(BF))
                for g in range(G):
                    for i, rr in enumerate(rows):
                        mid[g, rr, :] = r[i * N2:(i + 1) * N2, g * 128:(g + 1) * 128]
                return c
            lax.fori_loop(0, N // 128, s2, 0, unroll=U2)

            def s3(b, c):
                zz = jnp.concatenate(
                    [mid[g, pl.ds(b, N1, stride=P), :] for g in range(G)], axis=1)
                r = _dot(g1_ref[...], zz.astype(BF))
                for g in range(G):
                    ybuf[j * G + g, pl.ds(b, N1 // 2, stride=N2), :] = (
                        r[:, g * 128:(g + 1) * 128]
                        + uh[g, pl.ds(b, N1 // 2, stride=P), :]
                        * skt[j, 16:17, g * 128:(g + 1) * 128])
                return c
            lax.fori_loop(0, N2, s3, 0, unroll=U1)
            return carry

        lax.fori_loop(0, NT, tile, 0)

    pl.run_scoped(
        conv_phase,
        pltpu.VMEM((NT, S, CW), BF), pltpu.VMEM((NT, S, CW), BF),
        pltpu.VMEM((NT, CW, S), BF), pltpu.VMEM((S + 8, CW), F32),
        pltpu.VMEM((2 * G, N1 // 2 * P, 128), F32), pltpu.VMEM((2 * G, N1 * P, 128), F32),
        pltpu.VMEM((NT, 24, CW), F32))

    for c in big:
        c.wait()

    def mlp_phase(xbuf, zbuf, hs, obuf):
        hs[0:8, :] = jnp.zeros((8, D), F32)
        hs[S + 8:S + 16, :] = jnp.zeros((8, D), F32)

        def init(i, c):
            rows = pl.ds(pl.multiple_of(i * TM, TM), TM)
            xbuf[rows, :] = qbuf[rows, :].astype(F32)
            return c
        lax.fori_loop(0, S // TM, init, 0)

        def layer(l, carry):
            def pass_a(i, c):
                r0 = pl.multiple_of(i * TM, TM)
                rows = pl.ds(r0, TM)
                x = xbuf[rows, :]
                y = jnp.concatenate([ybuf[j, rows, :] for j in range(D // 128)], axis=1)
                x = x + _ln(x) * y
                xbuf[rows, :] = x
                z = _ln(x)
                zbuf[rows, :] = z
                h = _gelu(_dot(_ln(z).astype(BF), w1[...]))
                hs[pl.ds(r0 + 8, TM), :] = h
                return c
            lax.fori_loop(0, S // TM, pass_a, 0)

            def pass_b(i, c):
                r0 = pl.multiple_of(i * TM, TM)
                rows = pl.ds(r0, TM)
                C = D // 4
                parts = []
                for g, sh in enumerate((-1, 1, -2, 2)):
                    win = hs[pl.ds(r0, TM + 16), g * C:(g + 1) * C]
                    parts.append(win[8 + sh:8 + sh + TM].astype(BF))
                x1 = zbuf[rows, :] + _dot(jnp.concatenate(parts, axis=1), w2[...])
                xn = _ln(x1).astype(BF)
                acc = xbuf[rows, :] + x1
                for f in range(F // FC):
                    g = _gelu(_dot(xn, w3[:, f * FC:(f + 1) * FC])).astype(BF)
                    acc = acc + _dot(g, w4[f * FC:(f + 1) * FC, :])
                xbuf[rows, :] = acc

                @pl.when(l == 1)
                def _():
                    obuf[rows, :] = acc.astype(BF)
                    pltpu.make_async_copy(obuf.at[rows, :], o_hbm.at[0, rows, :], osem).start()
                return c
            lax.fori_loop(0, S // TM, pass_b, 0)
            return carry

        lax.fori_loop(0, 2, layer, 0)
        pltpu.make_async_copy(obuf, o_hbm.at[0], osem).wait()

    pl.run_scoped(
        mlp_phase,
        pltpu.VMEM((S, D), F32), pltpu.VMEM((S, D), F32),
        pltpu.VMEM((S + 16, D), F32), pltpu.VMEM((S, D), BF))


@jax.jit
def pallas_interleave_layers__ssm_conv_h3__mixer_s_mlp__prompt_kernel(
    A_q, A_k, A_v, A_shift_k, A_ssm_k, A_ssm_D, B_x, B_w1, B_w2, B_w3, B_w4,
):
    del B_x
    consts = [jnp.asarray(m.astype(BF)) for m in _dft_constants()]
    hbm = pl.BlockSpec(memory_space=pl.ANY)
    vmem = pl.BlockSpec(memory_space=pltpu.VMEM)
    return pl.pallas_call(
        _kernel,
        out_shape=jax.ShapeDtypeStruct((1, S, D), BF),
        in_specs=[hbm, hbm, hbm, vmem, hbm, vmem, vmem, vmem, vmem, vmem,
                  hbm, hbm, hbm, hbm],
        out_specs=hbm,
        scratch_shapes=[
            pltpu.VMEM((S, D), BF), pltpu.VMEM((D, D), BF), pltpu.VMEM((D, D), BF),
            pltpu.VMEM((D, F), BF), pltpu.VMEM((F, D), BF),
            pltpu.VMEM((D // 128, S, 128), F32),
            pltpu.SemaphoreType.DMA((3, NT)), pltpu.SemaphoreType.DMA((5,)),
            pltpu.SemaphoreType.DMA(()),
        ],
        compiler_params=pltpu.CompilerParams(vmem_limit_bytes=110 * 1024 * 1024),
    )(A_q, A_k, A_v, A_shift_k, A_ssm_k, A_ssm_D.reshape(1, D), *consts,
      B_w1, B_w2, B_w3, B_w4)
```

```python
import functools

import jax
import jax.numpy as jnp
import numpy as np
import jax.experimental.pallas as pl
import jax.experimental.pallas.tpu as pltpu
from jax import lax

S, D, F = 2048, 1024, 3584
KS = 4
N = 2 * S
N1 = 128
N2 = 32
CW = 256
NT = D // CW
G = CW // 128
P = 33
RB = 64
PY = 33
U1 = 8
U2 = 8
FA = 3
NS = 4
NL = 2
GC = 256
TM = 256
FC = 256
EPS = 1e-5
BF = jnp.bfloat16
F32 = jnp.float32


def _dft_constants():
    a = np.arange(N1 // 2)
    k1 = np.arange(N1 // 2)
    b = np.arange(N2)
    ang = -2 * np.pi * np.outer(k1 + 0.5, a) * N2 / N
    f1 = np.empty((N1, N1 // 2))
    f1[0::2], f1[1::2] = np.cos(ang), np.sin(ang)
    g1 = (2.0 / N) * f1.T
    grp = 64 // N2
    f2 = np.zeros((N1 // 2 // grp, 128, 128))
    for k in range(N1 // 2):
        an = -2 * np.pi * np.outer(k + 0.5 + N1 * b, b) / N
        c, s = np.cos(an), np.sin(an)
        p, g = divmod(k, grp)
        r, c0 = g * N2, g * 2 * N2
        f2[p, r:r + N2, c0:c0 + N2] = c
        f2[p, r:r + N2, c0 + N2:c0 + 2 * N2] = -s
        f2[p, 64 + r:64 + r + N2, c0:c0 + N2] = s
        f2[p, 64 + r:64 + r + N2, c0 + N2:c0 + 2 * N2] = c
    g2 = f2.transpose(0, 2, 1)
    return [np.ascontiguousarray(m).astype(np.float32) for m in (f1, f2, g2, g1)]


def _ln(x):
    m = jnp.mean(x, axis=-1, keepdims=True)
    c = x - m
    v = jnp.mean(c * c, axis=-1, keepdims=True)
    return c * lax.rsqrt(v + EPS)


def _gelu(x):
    inner = x * (0.7978845608028654 + 0.7978845608028654 * 0.044715 * (x * x))
    hx = 0.5 * x
    return hx + hx * jnp.tanh(inner)


def _dot(a, b):
    return jnp.dot(a, b, preferred_element_type=F32)


def _kernel(q_hbm, k_hbm, v_hbm, sk_ref, h_hbm, d_ref, f1_ref, f2_hbm, g2_hbm,
            g1_ref, w1_hbm, w2_hbm, w3_hbm, w4_hbm, o_hbm,
            qbuf, w1, w2, w3, w4, ybuf, csem, wsem, osem):
    def col_copies(j, kbuf, vbuf, hbuf):
        cols = pl.ds(j * CW, CW)
        return (
            pltpu.make_async_copy(k_hbm.at[0, :, cols], kbuf.at[j, pl.ds(16, S), :], csem.at[0, j]),
            pltpu.make_async_copy(v_hbm.at[0, :, cols], vbuf.at[j], csem.at[1, j]),
            pltpu.make_async_copy(h_hbm.at[cols, :], hbuf.at[j], csem.at[2, j]),
        )

    big = (
        pltpu.make_async_copy(q_hbm.at[0], qbuf, wsem.at[0]),
        pltpu.make_async_copy(w1_hbm, w1, wsem.at[1]),
        pltpu.make_async_copy(w2_hbm, w2, wsem.at[2]),
        pltpu.make_async_copy(w3_hbm, w3, wsem.at[3]),
        pltpu.make_async_copy(w4_hbm, w4, wsem.at[4]),
    )

    def conv_phase(kbuf, vbuf, hbuf, uh, mid, mid2, skt, f2_ref, g2_ref):
        tw = (pltpu.make_async_copy(f2_hbm, f2_ref, wsem.at[5]),
              pltpu.make_async_copy(g2_hbm, g2_ref, wsem.at[6]))
        for c in col_copies(0, kbuf, vbuf, hbuf) + col_copies(1, kbuf, vbuf, hbuf):
            c.start()
        for j in range(NT):
            skt[j, 0:KS, :] = sk_ref[:, j * CW:(j + 1) * CW].astype(F32)
            skt[j, 16:17, :] = d_ref[j * CW:(j + 1) * CW].astype(F32).reshape(1, CW)

        NQ = N // 128 // U2
        for j in range(NT):
            kbuf[j, 0:16, :] = jnp.zeros((16, CW), BF)

        def prep(j, sl, qi):
            for rr in range(S // RB // NQ):
                r = qi * (S // RB // NQ) + rr
                r0 = pl.multiple_of(r * RB, RB)
                kw = kbuf[j, pl.ds(r0, RB + 16), :].astype(F32)
                acc = None
                for t in range(KS):
                    term = kw[16 - t:16 - t + RB] * skt[j, t:t + 1, :]
                    acc = term if acc is None else acc + term
                u = acc * vbuf[j, pl.ds(r0, RB), :].astype(F32)
                for g in range(G):
                    for a in range(RB // N2):
                        uh[sl, g, pl.ds((r * (RB // N2) + a) * P, N2), :] = (
                            u[a * N2:(a + 1) * N2, g * 128:(g + 1) * 128])
            for rr in range(S // 128 // NQ):
                r = qi * (S // 128 // NQ) + rr
                ht = hbuf[j, :, pl.ds(pl.multiple_of(r * 128, 128), 128)].astype(F32).T
                for g in range(G):
                    for a in range(128 // N2):
                        uh[sl, G + g, pl.ds((r * (128 // N2) + a) * P, N2), :] = (
                            ht[a * N2:(a + 1) * N2, g * 128:(g + 1) * 128])

        for c in col_copies(0, kbuf, vbuf, hbuf):
            c.wait()
        for c in tw:
            c.start()

        def prep0(qi, c):
            prep(0, 0, qi)
            return c
        lax.fori_loop(0, NQ, prep0, 0)

        def tile(j, carry):
            sl = lax.rem(j, 2)

            def s1(b, c):
                x = jnp.concatenate(
                    [uh[sl, g, pl.ds(b, N1 // 2, stride=P), :] for g in range(2 * G)], axis=1)
                r = _dot(f1_ref[...], x.astype(BF))
                for g in range(2 * G):
                    mid[g, pl.ds(b, N1, stride=P), :] = r[:, g * 128:(g + 1) * 128]
                return c
            lax.fori_loop(0, N2, s1, 0, unroll=U1)

            for jj in range(NT):
                @pl.when(j == jj)
                def _():
                    if jj == 0:
                        for c in tw:
                            c.wait()
                    if jj + 1 < NT:
                        for c in col_copies(jj + 1, kbuf, vbuf, hbuf):
                            c.wait()
                    if jj + 2 < NT:
                        for c in col_copies(jj + 2, kbuf, vbuf, hbuf):
                            c.start()
                    for c in (big[0:1], big[1:3], big[3:4], big[4:5])[jj]:
                        c.start()

            def s2(pg, c):
                prep(jnp.minimum(j + 1, NT - 1), 1 - sl, pg)
                ys = []
                for pi in range(U2):
                    p = pg * U2 + pi
                    base = p * (128 // N2 * P)
                    rows = [pl.ds(base + i * P, N2) for i in range(128 // N2)]
                    m = jnp.concatenate(
                        [jnp.concatenate([mid[g, rr, :] for rr in rows], axis=0)
                         for g in range(2 * G)], axis=1)
                    z = _dot(f2_ref[p], m.astype(BF))
                    ur, ui = z[0:64, 0:CW], z[64:128, 0:CW]
                    hr, hi = z[0:64, CW:], z[64:128, CW:]
                    yv = jnp.concatenate([ur * hr - ui * hi, ur * hi + ui * hr], axis=0)
                    ys.append((p, rows, yv.astype(BF)))
                for p, rows, yv in ys:
                    r = _dot(g2_ref[p], yv)
                    for g in range(G):
                        for i, rr in enumerate(rows):
                            mid2[g, rr, :] = r[i * N2:(i + 1) * N2, g * 128:(g + 1) * 128]
                return c
            lax.fori_loop(0, N // 128 // U2, s2, 0)

            def s3(b, c):
                zz = jnp.concatenate(
                    [mid2[g, pl.ds(b, N1, stride=P), :] for g in range(G)], axis=1)
                r = _dot(g1_ref[...], zz.astype(BF))
                for g in range(G):
                    ybuf[j * G + g, pl.ds(b, N1 // 2, stride=PY), :] = (
                        r[:, g * 128:(g + 1) * 128]
                        + uh[sl, g, pl.ds(b, N1 // 2, stride=P), :]
                        * skt[j, 16:17, g * 128:(g + 1) * 128])
                return c
            lax.fori_loop(0, N2, s3, 0, unroll=U1)
            return carry

        lax.fori_loop(0, NT, tile, 0)

    pl.run_scoped(
        conv_phase,
        pltpu.VMEM((NT, S + 16, CW), BF), pltpu.VMEM((NT, S, CW), BF),
        pltpu.VMEM((NT, CW, S), BF),
        pltpu.VMEM((2, 2 * G, N1 // 2 * P, 128), F32), pltpu.VMEM((2 * G, N1 * P, 128), F32),
        pltpu.VMEM((G, N1 * P, 128), F32), pltpu.VMEM((NT, 24, CW), F32),
        pltpu.VMEM((N // 128, 128, 128), BF), pltpu.VMEM((N // 128, 128, 128), BF))

    for c in big[:3]:
        c.wait()

    def mlp_phase(xbuf, zbuf, hs, obuf, xnb):
        hs[0:8, :] = jnp.zeros((8, D), F32)
        hs[S + 8:S + 16, :] = jnp.zeros((8, D), F32)

        NR = S // TM

        def gate_norm(m):
            i = lax.rem(m, NR)
            outs = []
            for c in range(TM // GC):
                rows = pl.ds(pl.multiple_of(i * TM + c * GC, GC), GC)
                x = jnp.where(m < NR, qbuf[rows, :].astype(F32), xbuf[rows, :])
                y = jnp.concatenate([jnp.concatenate(
                    [ybuf[j, pl.ds((i * (TM // N2) + c * (GC // N2) + a) * PY, N2), :]
                     for a in range(GC // N2)], axis=0)
                    for j in range(D // 128)], axis=1)
                x = x + _ln(x) * y
                xbuf[rows, :] = x
                z = _ln(x)
                zbuf[rows, :] = z
                outs.append(_ln(z).astype(BF))
            return jnp.concatenate(outs, axis=0)

        def mix_in(m, zn):
            r0 = pl.multiple_of(lax.rem(m, NR) * TM, TM)
            hs[pl.ds(r0 + 8, TM), :] = _gelu(_dot(zn, w1[...]))

        def step(n, fuse):
            r0 = pl.multiple_of(lax.rem(n, NR) * TM, TM)
            rows = pl.ds(r0, TM)
            C = D // 4
            parts = []
            for g, sh in enumerate((-1, 1, -2, 2)):
                win = hs[pl.ds(r0, TM + 16), g * C:(g + 1) * C]
                parts.append(win[8 + sh:8 + sh + TM].astype(BF))
            x1 = zbuf[rows, :] + _dot(jnp.concatenate(parts, axis=1), w2[...])
            xn = _ln(x1).astype(BF)
            acc = xbuf[rows, :] + x1
            if fuse:
                zn = gate_norm(n + 2)
                if FA < 0:
                    mix_in(n + 2, zn)
            xnb[...] = xn

            def chunk(a, off, extra=None):
                g = _gelu(_dot(xnb[...], w3[:, pl.ds(off, FC)])).astype(BF)
                if extra is not None:
                    extra()
                return a + _dot(g, w4[pl.ds(off, FC), :])

            for f in range(NS):
                acc = chunk(acc, f * FC,
                            (lambda: mix_in(n + 2, zn)) if fuse and f == FA else None)
            xbuf[rows, :] = acc
            per = (F // FC - NS) // NL

            def hidden(t, c):
                a = xbuf[rows, :]
                for f in range(per):
                    a = chunk(a, pl.multiple_of((NS + t * per + f) * FC, FC))
                xbuf[rows, :] = a
                obuf[rows, :] = a.astype(BF)
                return c
            lax.fori_loop(0, NL, hidden, 0)

            @pl.when(n >= NR)
            def _():
                pltpu.make_async_copy(obuf.at[rows, :], o_hbm.at[0, rows, :], osem).start()

        def pro(m, c):
            mix_in(m, gate_norm(m))
            return c

        def main(n, c):
            step(n, True)
            return c

        def tail(n, c):
            step(n, False)
            return c

        lax.fori_loop(0, 2, pro, 0)
        for c in big[3:]:
            c.wait()
        lax.fori_loop(0, 2 * NR - 2, main, 0)
        lax.fori_loop(2 * NR - 2, 2 * NR, tail, 0)
        pltpu.make_async_copy(obuf, o_hbm.at[0], osem).wait()

    pl.run_scoped(
        mlp_phase,
        pltpu.VMEM((S, D), F32), pltpu.VMEM((S, D), F32),
        pltpu.VMEM((S + 16, D), F32), pltpu.VMEM((S, D), BF), pltpu.VMEM((TM, D), BF))


@jax.jit
def pallas_interleave_layers__ssm_conv_h3__mixer_s_mlp__prompt_kernel(
    A_q, A_k, A_v, A_shift_k, A_ssm_k, A_ssm_D, B_x, B_w1, B_w2, B_w3, B_w4,
):
    del B_x
    consts = [jnp.asarray(m.astype(BF)) for m in _dft_constants()]
    hbm = pl.BlockSpec(memory_space=pl.ANY)
    vmem = pl.BlockSpec(memory_space=pltpu.VMEM)
    return pl.pallas_call(
        _kernel,
        out_shape=jax.ShapeDtypeStruct((1, S, D), BF),
        in_specs=[hbm, hbm, hbm, vmem, hbm, vmem, vmem, hbm, hbm, vmem,
                  hbm, hbm, hbm, hbm],
        out_specs=hbm,
        scratch_shapes=[
            pltpu.VMEM((S, D), BF), pltpu.VMEM((D, D), BF), pltpu.VMEM((D, D), BF),
            pltpu.VMEM((D, F), BF), pltpu.VMEM((F, D), BF),
            pltpu.VMEM((D // 128, N1 // 2 * PY, 128), F32),
            pltpu.SemaphoreType.DMA((3, NT)), pltpu.SemaphoreType.DMA((7,)),
            pltpu.SemaphoreType.DMA(()),
        ],
        compiler_params=pltpu.CompilerParams(vmem_limit_bytes=110 * 1024 * 1024),
    )(A_q, A_k, A_v, A_shift_k.T, A_ssm_k, A_ssm_D, *consts,
      B_w1, B_w2, B_w3, B_w4)
```
